```python
import os as _os
_os.environ.setdefault("JAX_PLATFORMS", "cpu")
import jax
import jax.numpy as jnp

def _softmax(x, axis=-1):
    return jax.nn.softmax(x, axis=axis)
def _gelu(x):
    return jax.nn.gelu(x, approximate=True)
def _silu(x):
    return jax.nn.silu(x)
def _sigmoid(x):
    return jax.nn.sigmoid(x)
def _layernorm(x, axis=-1, eps=1e-5):
    m = jnp.mean(x, axis=axis, keepdims=True)
    v = jnp.var(x, axis=axis, keepdims=True)
    return (x - m) / jnp.sqrt(v + eps)
def _scatter_add(tgt, idx, src, axis=0):
    return tgt.at[idx].add(src)
def _segment_sum(src, seg, n):
    return jax.ops.segment_sum(src, seg, n)
class _Rng:
    def __init__(self, key):
        self._k = key
    def _next(self):
        self._k, sub = jax.random.split(self._k)
        return sub
    def normal(self, shape):
        return jax.random.normal(self._next(), shape, dtype=jnp.bfloat16)
    def randint(self, lo, hi, shape):
        return jax.random.randint(self._next(), shape, lo, hi, dtype=jnp.int32)
    def uniform(self, shape, lo=0.0, hi=1.0):
        return jax.random.uniform(self._next(), shape, jnp.bfloat16, lo, hi)
    def permutation(self, n):
        return jax.random.permutation(self._next(), n)


kernel_name = 'gated_mix__grouped_kv_mqa__glu_gated_reglu__prompt'

def setup_inputs():
    _rng = _Rng(jax.random.key(int.from_bytes(__import__("os").urandom(4), "little")))
    _w = (lambda a: (lambda t: t.astype(jnp.bfloat16) if jnp.issubdtype(t.dtype, jnp.floating) else t)(jnp.asarray(a)))
    def _A_setup():
        B, S, D, H = 1, 2048, 1024, 32
        Dh = D // H
        return {
            "x": _w((lambda *s: _rng.normal(s) * 0.05)(B, S, D)),
            "wq": _w((lambda *s: _rng.normal(s) * 0.2)(D, H * Dh)),
            "wk": _w((lambda *s: _rng.normal(s) * 0.2)(D, Dh)),
            "wv": _w((lambda *s: _rng.normal(s) * 0.05)(D, Dh)),
            "wo": _w((lambda *s: _rng.normal(s) * 0.05)(H * Dh, D)),
        }
    _A_in = _A_setup()

    def _B_setup():
        B, S, D, F = 1, 2048, 1024, 3584
        return {
            "x": _w((lambda *s: _rng.normal(s) * 0.05)(B, S, D)),
            "W_gate": _w((lambda *s: _rng.normal(s) * 0.8)(D, F) * (2.0 / D) ** 0.5),
            "W_up": _w((lambda *s: _rng.normal(s) * 0.8)(D, F) * (2.0 / D) ** 0.5),
            "W_down": _w((lambda *s: _rng.normal(s) * 0.8)(F, D) * (1.0 / F) ** 0.5),
        }
    _B_in = _B_setup()

    return {
        "A_x": _A_in["x"],
        "A_wq": _A_in["wq"],
        "A_wk": _A_in["wk"],
        "A_wv": _A_in["wv"],
        "A_wo": _A_in["wo"],
        "B_x": _B_in["x"],
        "B_W_gate": _B_in["W_gate"],
        "B_W_up": _B_in["W_up"],
        "B_W_down": _B_in["W_down"],
        "gate_w": _w((lambda *s: _rng.normal(s) * 0.05)(1024) * 16.0),
    }

def reference(A_x, A_wq, A_wk, A_wv, A_wo, B_x, B_W_gate, B_W_up, B_W_down, gate_w):
    def _A_ref(x, wq, wk, wv, wo):
        B, S, D = x.shape
        H = 32
        Dh = D // H
        q = (lambda x, *d: x.transpose(*d))((x @ wq).reshape(B, S, H, Dh), 0, 2, 1, 3)
        k = x @ wk
        v = x @ wv
        scores = jnp.einsum("bhqd,bkd->bhqk", q, k) * (Dh ** -0.5)
        p = _softmax(scores, axis=-1)
        o = jnp.einsum("bhqk,bkd->bhqd", p, v)
        return (lambda x, *d: x.transpose(*d))(o, 0, 2, 1, 3).reshape(B, S, H * Dh) @ wo

    def _B_ref(x, W_gate, W_up, W_down):
        gate = jnp.einsum("bsd,df->bsf", x, W_gate)
        up = jnp.einsum("bsd,df->bsf", x, W_up)
        gate = gate * (lambda x, dt: x.astype(dt))(gate > 0, gate.dtype)
        h = gate * up
        return jnp.einsum("bsf,fd->bsd", h, W_down)

    x = A_x
    g = _sigmoid((x * gate_w).sum(-1, keepdims=True))
    a = _A_ref(x, A_wq, A_wk, A_wv, A_wo)
    b = _B_ref(x, B_W_gate, B_W_up, B_W_down)
    return g * a + (1 - g) * b
```

```python
import functools
import math

import jax
import jax.numpy as jnp
from jax import lax
from jax.experimental import pallas as pl
from jax.experimental.pallas import tpu as pltpu

F32 = jnp.float32
BF16 = jnp.bfloat16

S = 2048
D = 1024
H = 32
DH = 32
F = 3584

W = 512
KC = 128
U = 4
NQB = S // W
NB = NQB * H // U

NT_DIMS = (((1,), (1,)), ((), ()))


def _dot(a, b):
    return jnp.dot(a, b, preferred_element_type=F32)


def _kernel(x_hbm, wq_hbm, wkt_hbm, wvt_hbm, wo_hbm, wg_hbm, wu_hbm, wd_hbm, gw_hbm,
            out_hbm,
            x_v, wq_v, wt_v, gw_v, wo_v, wg_v, wu_v, wd_v,
            k_v, vt_v, qt_v, grow_v, gcol_v, ot_v, out_v, sems):
    cp_small = [
        pltpu.make_async_copy(wkt_hbm, wt_v.at[pl.ds(D, DH)], sems.at[0]),
        pltpu.make_async_copy(wvt_hbm, wt_v.at[pl.ds(D + DH, DH)], sems.at[1]),
        pltpu.make_async_copy(gw_hbm, gw_v, sems.at[2]),
    ]
    cp_wq = pltpu.make_async_copy(wq_hbm, wq_v, sems.at[3])
    cp_x = [
        pltpu.make_async_copy(x_hbm.at[pl.ds(c * W, W)], x_v.at[pl.ds(c * W, W)],
                              sems.at[4 + c])
        for c in range(NQB)
    ]
    cp_ffn = [
        pltpu.make_async_copy(wg_hbm, wg_v, sems.at[8]),
        pltpu.make_async_copy(wu_hbm, wu_v, sems.at[9]),
        pltpu.make_async_copy(wo_hbm, wo_v, sems.at[10]),
        pltpu.make_async_copy(wd_hbm, wd_v, sems.at[11]),
    ]
    cp_wq.start()
    for c in cp_small:
        c.start()
    for c in cp_x:
        c.start()

    cp_wq.wait()
    for j in range(D // 128):
        wt_v[pl.ds(j * 128, 128), :] = wq_v[:, pl.ds(j * 128, 128)].T
    for c in cp_small:
        c.wait()
    gw = gw_v[...].astype(F32)
    for j in range(D // 128):
        wt_v[pl.ds(D + 2 * DH, 16), pl.ds(j * 128, 128)] = jnp.broadcast_to(
            gw[j:j + 1, :], (16, 128)).astype(BF16)

    q_scale = DH ** -0.5 * math.log2(math.e)
    for c in range(NQB):
        cp_x[c].wait()
        if c == NQB - 1:
            for cp in cp_ffn:
                cp.start()
        rows = pl.ds(c * W, W)
        r = lax.dot_general(wt_v[...], x_v[rows, :], NT_DIMS,
                            preferred_element_type=F32)
        qt_v[c] = (r[:D] * q_scale).astype(BF16)
        kvt = r[D:D + 2 * DH]
        vt_v[:, rows] = kvt[DH:].astype(BF16)
        kpad = jnp.concatenate([kvt, jnp.zeros((128 - 2 * DH, W), F32)], axis=0)
        k_v[rows, :] = kpad.T[:, :DH].astype(BF16)
        g = jax.nn.sigmoid(r[D + 2 * DH:D + 2 * DH + 8])
        grow_v[c] = g
        gcol_v[rows, :] = jnp.broadcast_to(1.0 - g[:1], (128, W)).T

    def attention(sa, sb, m_v):
        def block(b_next, b_cur, s_w, s_r, pw, pr, do_qk=True, do_pv=True):
            def loc(b, u):
                return b // (H // U), pl.ds(
                    pl.multiple_of(((b % (H // U)) * U + u) * DH, DH), DH)

            for u in range(U):
                if do_qk:
                    qb, hs = loc(b_next, u)
                    qt = qt_v[qb, hs, :]
                if do_pv:
                    m_cur = m_v[pr, u]
                m_new = l = acc = None
                for c in range(S // KC):
                    ks = pl.ds(c * KC, KC)
                    if do_qk:
                        s = _dot(k_v[ks, :], qt)
                        s_w[u, ks, :] = s
                        mm = s.reshape(KC // 8, 8, W).max(axis=0)
                        m_new = mm if m_new is None else jnp.maximum(m_new, mm)
                    if do_pv:
                        p = jnp.exp2(s_r[u, ks, :].reshape(KC // 8, 8, W) - m_cur[None])
                        ls = p.sum(axis=0)
                        l = ls if l is None else l + ls
                        o = _dot(vt_v[:, ks], p.reshape(KC, W).astype(BF16))
                        acc = o if acc is None else acc + o
                if do_pv:
                    qb, hs = loc(b_cur, u)
                    scale = grow_v[qb][:1] / jnp.sum(l, axis=0, keepdims=True)
                    ot_v[qb, hs, :] = (acc * scale).astype(BF16)
                if do_qk:
                    m_v[pw, u] = jnp.broadcast_to(
                        jnp.max(m_new, axis=0, keepdims=True), (8, W))

        block(0, None, sa, None, 0, None, do_pv=False)

        def body(i, _):
            @pl.when(i % 2 == 0)
            def _():
                block(i + 1, i, sb, sa, 1, 0)

            @pl.when(i % 2 == 1)
            def _():
                block(i + 1, i, sa, sb, 0, 1)

        lax.fori_loop(0, NB - 1, body, None)
        block(None, NB - 1, None, sb, None, 1, do_qk=False)

    pl.run_scoped(attention, pltpu.VMEM((U, S, W), F32), pltpu.VMEM((U, S, W), F32),
                  pltpu.VMEM((2, U, 8, W), F32))

    for cp in cp_ffn:
        cp.wait()

    def ffn(h_v, o_v):
        TF = 512
        nf = F // TF

        def up_body(r, _):
            rows = pl.ds(pl.multiple_of(r * W, W), W)
            o_v[rows, :] = ot_v[r].T
            gc = gcol_v[rows, :]
            for f in range(nf):
                cols = pl.ds(f * TF, TF)
                xr = x_v[rows, :]
                gate = _dot(xr, wg_v[:, cols])
                up = _dot(xr, wu_v[:, cols])
                h = jnp.where(gate > 0, gate, 0.0) * up * jnp.tile(gc, (1, TF // 128))
                h_v[rows, cols] = h.astype(BF16)

        lax.fori_loop(0, S // W, up_body, None)

        TM = 256

        def out_copy(r):
            rows = pl.ds(pl.multiple_of(r * TM, TM), TM)
            return pltpu.make_async_copy(out_v.at[rows], out_hbm.at[rows], sems.at[12 + r])

        def down_body(r, _):
            rows = pl.ds(pl.multiple_of(r * TM, TM), TM)
            y = _dot(h_v[rows, :], wd_v[...]) + _dot(o_v[rows, :], wo_v[...])
            out_v[rows, :] = y.astype(BF16)
            out_copy(r).start()

        lax.fori_loop(0, S // TM, down_body, None)
        for r in range(S // TM):
            out_copy(r).wait()

    pl.run_scoped(ffn, pltpu.VMEM((S, F), BF16), pltpu.VMEM((S, D), BF16))


@jax.jit
def pallas_gated_mix__grouped_kv_mqa__glu_gated_reglu__prompt_kernel(
    A_x, A_wq, A_wk, A_wv, A_wo, B_x, B_W_gate, B_W_up, B_W_down, gate_w,
):
    del B_x
    any_spec = pl.BlockSpec(memory_space=pl.ANY)
    out = pl.pallas_call(
        _kernel,
        out_shape=jax.ShapeDtypeStruct((S, D), BF16),
        in_specs=[any_spec] * 9,
        out_specs=any_spec,
        scratch_shapes=[
            pltpu.VMEM((S, D), BF16),
            pltpu.VMEM((D, D), BF16),
            pltpu.VMEM((D + 2 * DH + 16, D), BF16),
            pltpu.VMEM((8, 128), BF16),
            pltpu.VMEM((D, D), BF16),
            pltpu.VMEM((D, F), BF16),
            pltpu.VMEM((D, F), BF16),
            pltpu.VMEM((F, D), BF16),
            pltpu.VMEM((S, DH), BF16),
            pltpu.VMEM((DH, S), BF16),
            pltpu.VMEM((NQB, D, W), BF16),
            pltpu.VMEM((NQB, 8, W), F32),
            pltpu.VMEM((S, 128), F32),
            pltpu.VMEM((NQB, D, W), BF16),
            pltpu.VMEM((S, D), BF16),
            pltpu.SemaphoreType.DMA((20,)),
        ],
        compiler_params=pltpu.CompilerParams(vmem_limit_bytes=120 * 2**20),
        name="gated_mix",
    )(
        A_x.reshape(S, D), A_wq, A_wk.T, A_wv.T, A_wo, B_W_gate, B_W_up, B_W_down,
        gate_w.reshape(8, 128),
    )
    return out.reshape(1, S, D)
```

```python
import functools
import itertools
import math

import jax
import jax.numpy as jnp
from jax import lax
from jax.experimental import pallas as pl
from jax.experimental.pallas import tpu as pltpu

F32 = jnp.float32
BF16 = jnp.bfloat16

S = 2048
D = 1024
H = 32
DH = 32
F = 3584

W = S // 4
KC = 128
G = 8
HT = D // 128
NCH = F // 512
PHASES = "PATUD"
KV = 32

L_MIN, L_MAX, V_MAX = 2.0 ** -20, 2.0 ** 40, 2.0 ** 80

NT_DIMS = (((1,), (1,)), ((), ()))

SU = ({(0, 0): 1, (1, 1): 1}, {(1, 0): 1, (1, 1): 1}, {(0, 0): 1}, {(1, 1): 1},
      {(0, 0): 1, (0, 1): 1}, {(1, 0): 1, (0, 0): -1}, {(0, 1): 1, (1, 1): -1})
SV = ({(0, 0): 1, (1, 1): 1}, {(0, 0): 1}, {(0, 1): 1, (1, 1): -1},
      {(1, 0): 1, (0, 0): -1}, {(1, 1): 1}, {(0, 0): 1, (0, 1): 1},
      {(1, 0): 1, (1, 1): 1})
SW = ({(0, 0): 1, (1, 1): 1}, {(1, 0): 1, (1, 1): -1}, {(0, 1): 1, (1, 1): 1},
      {(0, 0): 1, (1, 0): 1}, {(0, 0): -1, (0, 1): 1}, {(1, 1): 1}, {(0, 0): 1})
ORDER = (1, 3, 0, 2, 4, 5, 6)
QUADS = ((1, 0), (0, 1), (1, 1), (0, 0))


def _dot(a, b):
    return jnp.dot(a, b, preferred_element_type=F32)


def _tree(op, xs):
    while len(xs) > 1:
        xs = [functools.reduce(op, xs[i:i + 2]) for i in range(0, len(xs), 2)]
    return xs[0]


def _signed_sum(terms):
    terms = sorted(terms, key=lambda t: -t[0])
    acc = terms[0][1] if terms[0][0] > 0 else -terms[0][1]
    for sign, v in terms[1:]:
        acc = acc + v if sign > 0 else acc - v
    return acc


def _operand(table, p, q, block):
    terms = [(s * t, block(2 * a + c, 2 * b + d))
             for (a, b), s in table[p].items() for (c, d), t in table[q].items()]
    if len(terms) == 1:
        return terms[0][1].astype(BF16)
    return _signed_sum([(s, v.astype(F32)) for s, v in terms]).astype(BF16)


def _strassen2(outer, product, emit, acc_ref=None):
    before = ORDER[:ORDER.index(outer[0])]
    terms = {}
    for n, p in enumerate(outer):
        inner = {q: product(p, q) for q in ORDER}
        later = ORDER[len(before) + n + 1:]
        for i2, j2 in QUADS:
            v = _signed_sum([(SW[q][i2, j2], m) for q, m in inner.items()
                             if (i2, j2) in SW[q]])
            for (i1, j1), sign in SW[p].items():
                i, j = 2 * i1 + i2, 2 * j1 + j2
                terms.setdefault((i, j), []).append((sign, v))
                if not any((i1, j1) in SW[r] for r in later):
                    parts = terms.pop((i, j))
                    if any((i1, j1) in SW[r] for r in before):
                        parts = [(1, acc_ref[i, j])] + parts
                    emit(i, j, _signed_sum(parts))
    for (i, j), parts in terms.items():
        if any((i // 2, j // 2) in SW[r] for r in before):
            parts = [(1, acc_ref[i, j])] + parts
        acc_ref[i, j] = _signed_sum(parts)


def _kernel(x_hbm, wq_hbm, wkt_hbm, wvt_hbm, wo_hbm, wg_hbm, wu_hbm, wd_hbm, gw_hbm,
            out_hbm,
            wo_v, wg_v, wu_v, wd_v, grow_v, gcol_v, o_v, flag, sems, xa_v):
    flag[0] = 1
    new_block = lambda fn: pl.when(flag[0] == 1)(fn)
    cp_ffn = [
        pltpu.make_async_copy(wg_hbm, wg_v, sems.at[10]),
        pltpu.make_async_copy(wu_hbm, wu_v, sems.at[11]),
        pltpu.make_async_copy(wo_hbm, wo_v, sems.at[12]),
        pltpu.make_async_copy(wd_hbm, wd_v, sems.at[13]),
    ]

    def up_chunk(c0, store_h, hook=None):
        def wblock(k, j):
            rs, cs = pl.ds(k * 256, 256), pl.ds(c0 + j * 128, 128)
            return jnp.concatenate([wg_v[rs, cs], wu_v[rs, cs]], axis=1)

        def product(p, q):
            if hook is not None:
                hook()
            return _dot(xa_v[7 * p + q], _operand(SV, p, q, wblock))

        def emit(i, j, v):
            store_h(j, i, jnp.maximum(v[:, :128], 0.0) * v[:, 128:] * gcol_v[i])

        _strassen2(ORDER, product, emit)

    def attention_branch(qt_v, k_v, kb_v, vt_v, p_v, l_v, ot_v, rng_v):
        def query_tile(n):
            hs = pl.ds(pl.multiple_of((n % H) * DH, DH), DH)
            return qt_v[query_block(n), hs, :]

        def query_block(n):
            return (n // H + 2) % 4

        def key_column(c, r):
            return [kb_v[c, d, pl.ds(r - (KC - KV), 8)] for d in range(DH)]

        def new_key_column(c, r):
            k = k_v[pl.ds(c * KC + r // 16 * 16, 16), :].astype(F32)[r % 16:r % 16 + 8]
            cols = [jnp.broadcast_to(k[:, d:d + 1], (8, 128)) for d in range(DH)]
            for d in range(DH):
                kb_v[c, d, pl.ds(r - (KC - KV), 8)] = cols[d]
            return cols

        def weights(n, u, first):
            qt = query_tile(n)
            t0 = u % 4
            qf = qt[:, t0 * 128:(t0 + 1) * 128].astype(F32)
            qd = [jnp.broadcast_to(qf[d:d + 1], (8, 128)) for d in range(DH)]
            l = [None] * 4
            for c in range(S // KC):
                lo, hi = KC - KV, KC
                if first:
                    lo += u // 4 * KV // 2
                    hi = lo + (KV // 2 if c % 4 == t0 else 0)
                rows = []
                for t in range(4):
                    spans = [(0, lo), (hi, KC)] if t == t0 else [(0, KC)]
                    k = jnp.concatenate([k_v[pl.ds(c * KC + a, b - a), :]
                                         for a, b in spans if b > a], axis=0)
                    p = jnp.exp2(_dot(k, qt[:, t * 128:(t + 1) * 128]))
                    rows.append([p[r:r + 8] for r in range(0, p.shape[0], 8)])
                extra = []
                for r in range(lo, hi, 8):
                    kd = new_key_column(c, r) if first else key_column(c, r)
                    extra.append(jnp.exp2(functools.reduce(
                        jnp.add, [qd[d] * kd[d] for d in range(DH)])))
                tiles = [r[:lo // 8] + extra + r[lo // 8:] if t == t0 else r
                         for t, r in enumerate(rows)]
                p_v[u, pl.ds(c * KC, KC), :] = jnp.concatenate(
                    [jnp.concatenate(r, axis=0) for r in tiles], axis=1).astype(BF16)
                for z, e in enumerate(extra):
                    r = len(rows[t0]) * z // len(extra) + 1
                    rows[t0][r] = rows[t0][r] + e
                for t in range(4):
                    if c > 0:
                        rows[t][0] = rows[t][0] + l[t]
                    l[t] = _tree(jnp.add, rows[t])
                if c == S // KC - 1:
                    l_v[u] = jnp.concatenate(l, axis=1)
                yield

        def outputs(n, u):
            if u % 4 == 0:
                store_o(jnp.maximum(n // 4 - 1, 0), (u // 4 + 1) % 2)
            l = jnp.sum(l_v[u], axis=0, keepdims=True)
            for c in range(S // KC):
                p = p_v[u, pl.ds(c * KC, KC), :]
                yield
                o = _dot(vt_v[c * KC // W, :, pl.ds(c * KC % W, KC)], p)
                acc = o if c == 0 else acc + o
                if c == S // KC - 1:
                    g = grow_v[query_block(n)][:1]
                    ot_v[u // 4, pl.ds(u % 4 * DH, DH), :] = acc * (g / l)
                    in_range = jnp.logical_and(l >= L_MIN, l <= L_MAX)
                    rng_v[...] = jnp.where(in_range, rng_v[...], 1.0)
                yield

        def store_o(t, slot):
            o_v[t % HT, query_block(4 * t)] = ot_v[slot].T

        def group(n, do_out=True, do_new=True):
            outs = itertools.chain(*[outputs(n + u, u) for u in range(G) if do_out])
            news = itertools.chain(*[weights(n + G + u, u, not do_out)
                                     for u in range(G) if do_new])
            for _ in range(G * S // KC):
                next(outs, None)
                next(news, None)
                next(outs, None)

        def stripe_with_max(n, _):
            qt = query_tile(n)

            def keys(c, carry):
                m, l, acc = carry
                s = _dot(k_v[pl.ds(pl.multiple_of(c * W, W), W), :], qt)
                m_new = jnp.maximum(m, jnp.max(s, axis=0, keepdims=True))
                alpha = jnp.exp2(m - m_new)
                p = jnp.exp2(s - m_new)
                return (m_new, alpha * l + jnp.sum(p, axis=0, keepdims=True),
                        alpha * acc + _dot(vt_v[c], p.astype(BF16)))

            _, l, acc = lax.fori_loop(
                0, S // W, keys,
                (jnp.full((1, W), jnp.finfo(F32).min, F32), jnp.zeros((1, W), F32),
                 jnp.zeros((DH, W), F32)))
            hs = pl.ds(pl.multiple_of((n % 4) * DH, DH), DH)
            ot_v[0, hs, :] = acc * (grow_v[query_block(n)][:1] / l)
            pl.when(n % 4 == 3)(lambda: store_o(n // 4, 0))

        def project(x_v, wq_v, wt_v, gw_v, acc_v, xf_v, early_v):
            def copy(src, dst, idx, sem):
                return pltpu.make_async_copy(src.at[idx], dst.at[idx], sems.at[sem])

            cp_small = [
                pltpu.make_async_copy(wkt_hbm, wt_v.at[pl.ds(0, DH)], sems.at[0]),
                pltpu.make_async_copy(wvt_hbm, wt_v.at[pl.ds(DH, DH)], sems.at[1]),
                pltpu.make_async_copy(gw_hbm, gw_v, sems.at[2]),
            ]
            cp_x = [copy(x_hbm, x_v, pl.ds(i * W, W), 3 + i) for i in range(4)]
            cp_wq = [copy(wq_hbm, wq_v, (slice(None), pl.ds(c0, cn)), 7 + j)
                     for j, (c0, cn) in enumerate([(0, 256), (256, 256), (512, 512)])]
            for cp in cp_small + [cp_x[3], cp_wq[0], cp_x[2], cp_wq[1], cp_x[0], cp_x[1],
                                  cp_wq[2]]:
                cp.start()
            ot_v[1] = jnp.zeros(ot_v.shape[1:], F32)
            rng_v[...] = jnp.zeros(rng_v.shape, F32)
            with jax.named_scope("wait0"):
                for cp in cp_small:
                    cp.wait()
            gw = gw_v[...].astype(F32)
            for j in range(D // 128):
                wt_v[pl.ds(2 * DH, 16), pl.ds(j * 128, 128)] = jnp.broadcast_to(
                    gw[j:j + 1, :], (16, 128)).astype(BF16)

            def kv(i):
                rows = pl.ds(i * W, W)
                xf_v[rows, :] = x_v[rows, :].astype(F32)
                r = lax.dot_general(wt_v[...], x_v[rows, :], NT_DIMS,
                                    preferred_element_type=F32)
                vt_v[i] = r[DH:2 * DH].astype(BF16)
                kpad = jnp.concatenate([r[:DH], jnp.zeros((128 - DH, W), F32)], axis=0)
                k_v[rows, :] = kpad.T[:, :DH].astype(BF16)
                v_peak = jnp.max(jnp.abs(r[DH:2 * DH]), axis=0, keepdims=True)
                rng_v[...] = jnp.where(v_peak <= V_MAX, rng_v[...], 1.0)
                g = jax.nn.sigmoid(r[2 * DH:2 * DH + 8])
                grow_v[i] = g
                gcol_v[i] = jnp.broadcast_to(1.0 - g[:1], (128, W)).T

            early = [(1, 1), (1, 3), (3, 1), (3, 3)]

            def product(p, q):
                if (p, q) in early:
                    return early_v[early.index((p, q))]
                return new_product(p, q)

            def new_product(p, q):
                a = _operand(SU, p, q,
                             lambda i, k: xf_v[pl.ds(i * W, W), pl.ds(k * 256, 256)])
                xa_v[7 * p + q] = a
                return _dot(xa_v[7 * p + q], _operand(
                    SV, p, q, lambda k, j: wq_v[pl.ds(k * 256, 256), pl.ds(j * 256, 256)]))

            def emit(i, j, v):
                q_scale = DH ** -0.5 * math.log2(math.e)
                qt_v[i, pl.ds(j * 256, 256), :] = (v.T * q_scale).astype(BF16)

            with jax.named_scope("wait1"):
                cp_x[3].wait()
            kv(3)
            with jax.named_scope("wait2"):
                cp_wq[0].wait()

            @new_block
            def _():
                for j, (p, q) in enumerate(early):
                    early_v[j] = new_product(p, q)

            with jax.named_scope("wait3"):
                cp_x[2].wait()
                cp_wq[1].wait()

            @new_block
            def _():
                kv(2)
                _strassen2(ORDER[:2], product, emit, acc_v)

            with jax.named_scope("wait4"):
                for cp in (cp_x[0], cp_x[1], cp_wq[2]):
                    cp.wait()
            for cp in cp_ffn:
                cp.start()

            @new_block
            def _():
                kv(0)
                kv(1)
                _strassen2(ORDER[2:4], product, emit, acc_v)

            @new_block
            def _():
                _strassen2(ORDER[4:], product, emit, acc_v)
                group(-G, do_out=False)

        if "P" in PHASES:
          with jax.named_scope("proj"):
            pl.run_scoped(project, pltpu.VMEM((S, D), BF16), pltpu.VMEM((D, D), BF16),
                          pltpu.VMEM((2 * DH + 16, D), BF16), pltpu.VMEM((8, 128), BF16),
                          pltpu.VMEM((4, 4, W, 256), F32), pltpu.VMEM((S, D), F32),
                          pltpu.VMEM((4, W, 256), F32))

        n_groups = 4 * H // G
        if "A" in PHASES:
          with jax.named_scope("att_loop"):
            lax.fori_loop(0, n_groups - 1, lambda i, _: group(i * G), None)
        if "T" in PHASES:
          with jax.named_scope("att_tail"):
            group((n_groups - 1) * G, do_new=False)
            store_o(4 * HT - 1, 1)

            @pl.when(jnp.max(rng_v[...]) > 0.0)
            def _():
                lax.fori_loop(0, 4 * H, stripe_with_max, None)
        else:
            z = flag[0]
            o_v[z, z] = (p_v[z, pl.ds(z * 512, 512), :128].astype(F32) + kb_v[z, z, :1] + rng_v[:1, :128] + l_v[z][:1, :128] + ot_v[z, :1, :128] + grow_v[z, :1, :128]
                         + vt_v[z][:1, :128].astype(F32) + qt_v[z, :512, :128].astype(F32))

    pl.run_scoped(attention_branch, pltpu.VMEM((4, D, W), BF16),
                  pltpu.VMEM((S, DH), BF16), pltpu.VMEM((S // KC, DH, KV, 128), F32),
                  pltpu.VMEM((4, DH, W), BF16), pltpu.VMEM((G, S, W), BF16),
                  pltpu.VMEM((G, 8, W), F32), pltpu.VMEM((2, 128, W), F32),
                  pltpu.VMEM((1, W), F32))

    def ffn(h_v, acc_v):
        if "P" in PHASES:
          for cp in cp_ffn:
            cp.wait()

        def up_body(c, _):
            def store_h(j, i, v):
                h_v[4 * c + j, i] = v

            up_chunk(pl.multiple_of(c * 512, 512), store_h)

        if "U" in PHASES:
          with jax.named_scope("up"):
            lax.fori_loop(0, NCH, up_body, None)

        def hblock(i, k):
            return jnp.concatenate(
                [h_v[4 * t + k, i] for t in range(NCH)]
                + [o_v[4 * t + k, i] for t in range(D // 512)], axis=1)

        def wblock(k, j):
            cs = pl.ds(j * 256, 256)
            return jnp.concatenate(
                [wd_v[pl.ds((4 * t + k) * 128, 128), cs] for t in range(NCH)]
                + [wo_v[pl.ds((4 * t + k) * 128, 128), cs] for t in range(D // 512)],
                axis=0)

        def staging(i, j):
            return wg_v.at[pl.ds(i % 2 * W, W), pl.ds(i // 2 * D + j * 256, 256)]

        def out_copy(i, j):
            return pltpu.make_async_copy(
                staging(i, j), out_hbm.at[pl.ds(i * W, W), pl.ds(j * 256, 256)],
                sems.at[14 + 4 * i + j])

        def down_product(p, q):
            return _dot(_operand(SU, p, q, hblock), _operand(SV, p, q, wblock))

        def last_stage():
            p = ORDER[-1]
            inner = {q: down_product(p, q) for q in ORDER[:-1]}
            for i, j in QUADS:
                v = _signed_sum([(1, acc_v[i, j])] + [
                    (SW[q][i, j], m) for q, m in inner.items() if (i, j) in SW[q]])
                if (i, j) == (0, 0):
                    acc_v[i, j] = v
                else:
                    staging(i, j)[...] = v.astype(BF16)
            for i, j in QUADS[:-1]:
                out_copy(i, j).start()

        def last_product():
            v = acc_v[0, 0] + down_product(ORDER[-1], ORDER[-1])
            staging(0, 0)[...] = v.astype(BF16)
            out_copy(0, 0).start()

        def down_stage(p):
            done = []

            def emit(i, j, v):
                staging(i, j)[...] = v.astype(BF16)
                done.append((i, j))

            _strassen2((p,), down_product, emit, acc_v)
            for i, j in done:
                out_copy(i, j).start()

        if "D" not in PHASES:
            z = flag[0]
            wg_v[:512, :128] = xa_v[z, :, :128] + (h_v[z, z] + o_v[z, z] + gcol_v[z]).astype(BF16)
            cp = out_copy(0, 1); cp.start(); cp.wait()
        if "D" in PHASES:
          with jax.named_scope("down"):
            for p in ORDER[:-1]:
                new_block(functools.partial(down_stage, p))
            new_block(last_stage)
            new_block(last_product)
          with jax.named_scope("wait_out"):
            for i in range(4):
                for j in range(4):
                    out_copy(i, j).wait()

    pl.run_scoped(ffn, pltpu.VMEM((4 * NCH, 4, W, 128), F32),
                  pltpu.VMEM((4, 4, W, 256), F32))


def _entry(*refs):
    pl.run_scoped(functools.partial(_kernel, *refs), pltpu.VMEM((49, W, D // 4), BF16))


@jax.jit
def pallas_gated_mix__grouped_kv_mqa__glu_gated_reglu__prompt_kernel(
    A_x, A_wq, A_wk, A_wv, A_wo, B_x, B_W_gate, B_W_up, B_W_down, gate_w,
):
    del B_x
    any_spec = pl.BlockSpec(memory_space=pl.ANY)
    out = pl.pallas_call(
        _entry,
        out_shape=jax.ShapeDtypeStruct((S, D), BF16),
        in_specs=[any_spec] * 9,
        out_specs=any_spec,
        scratch_shapes=[
            pltpu.VMEM((D, D), BF16),
            pltpu.VMEM((D, F), BF16),
            pltpu.VMEM((D, F), BF16),
            pltpu.VMEM((F, D), BF16),
            pltpu.VMEM((4, 8, W), F32),
            pltpu.VMEM((4, W, 128), F32),
            pltpu.VMEM((HT, 4, W, 128), F32),
            pltpu.SMEM((1,), jnp.int32),
            pltpu.SemaphoreType.DMA((30,)),
        ],
        compiler_params=pltpu.CompilerParams(vmem_limit_bytes=127 * 2**20),
        name="gated_mix",
    )(
        A_x.reshape(S, D), A_wq, A_wk.T, A_wv.T, A_wo, B_W_gate, B_W_up, B_W_down,
        gate_w.reshape(8, 128),
    )
    return out.reshape(1, S, D)
```

```python
import functools
import itertools
import math

import jax
import jax.numpy as jnp
from jax import lax
from jax.experimental import pallas as pl
from jax.experimental.pallas import tpu as pltpu

F32 = jnp.float32
BF16 = jnp.bfloat16

S = 2048
D = 1024
H = 32
DH = 32
F = 3584

W = S // 4
G = 8
KC = 128
NKC = S // KC
KV = 32
KM = KC - KV
KV0 = NKC * KM
HT = D // 128
NCH = F // 512

L_MIN, L_MAX, V_MAX = 2.0 ** -20, 2.0 ** 40, 2.0 ** 80

SU = ({(0, 0): 1, (1, 1): 1}, {(1, 0): 1, (1, 1): 1}, {(0, 0): 1}, {(1, 1): 1},
      {(0, 0): 1, (0, 1): 1}, {(1, 0): 1, (0, 0): -1}, {(0, 1): 1, (1, 1): -1})
SV = ({(0, 0): 1, (1, 1): 1}, {(0, 0): 1}, {(0, 1): 1, (1, 1): -1},
      {(1, 0): 1, (0, 0): -1}, {(1, 1): 1}, {(0, 0): 1, (0, 1): 1},
      {(1, 0): 1, (1, 1): 1})
SW = ({(0, 0): 1, (1, 1): 1}, {(1, 0): 1, (1, 1): -1}, {(0, 1): 1, (1, 1): 1},
      {(0, 0): 1, (1, 0): 1}, {(0, 0): -1, (0, 1): 1}, {(1, 1): 1}, {(0, 0): 1})
QUADS = ((1, 0), (0, 1), (1, 1), (0, 0))
OUTER, INNER = (1, 3, 0, 2, 4, 5, 6), (1, 0, 2, 4, 3, 5, 6)
OUTER_UP, INNER_UP = (1, 5, 3, 0, 2, 4, 6), (1, 2, 3, 4, 0, 5, 6)


def _dot(a, b):
    return jnp.dot(a, b, preferred_element_type=F32)


def _tree_sum(xs):
    while len(xs) > 1:
        xs = [functools.reduce(jnp.add, xs[i:i + 2]) for i in range(0, len(xs), 2)]
    return xs[0]


def _signed_sum(terms):
    terms = sorted(terms, key=lambda t: -t[0])
    acc = terms[0][1] if terms[0][0] > 0 else -terms[0][1]
    for sign, v in terms[1:]:
        acc = acc + v if sign > 0 else acc - v
    return acc


def _operand(table, p, q, block):
    terms = [(s * t, block(2 * a + c, 2 * b + d))
             for (a, b), s in table[p].items() for (c, d), t in table[q].items()]
    if len(terms) == 1:
        return terms[0][1].astype(BF16)
    return _signed_sum([(s, v.astype(F32)) for s, v in terms]).astype(BF16)


def _strassen2(part, product, emit, acc_ref=None, outer=OUTER, inner=INNER):
    before = outer[:outer.index(part[0])]

    def total(i, j, terms):
        if any((i // 2, j // 2) in SW[r] for r in before):
            terms = [(1, acc_ref[i, j])] + terms
        return _signed_sum(terms)

    pending = {}
    for n, p in enumerate(part):
        prods = {q: product(p, q) for q in inner}
        later = outer[len(before) + n + 1:]
        for i2, j2 in QUADS:
            v = _signed_sum([(SW[q][i2, j2], m) for q, m in prods.items()
                             if (i2, j2) in SW[q]])
            for (i1, j1), sign in SW[p].items():
                i, j = 2 * i1 + i2, 2 * j1 + j2
                pending.setdefault((i, j), []).append((sign, v))
                if not any((i1, j1) in SW[r] for r in later):
                    emit(i, j, total(i, j, pending.pop((i, j))))
    for (i, j), terms in pending.items():
        acc_ref[i, j] = total(i, j, terms)


def _kernel(x_hbm, wq_hbm, wkt_hbm, wvt_hbm, wo_hbm, wg_hbm, wu_hbm, wd_hbm, gw_hbm,
            out_hbm, wo_v, wg_v, wu_v, wd_v, grow_v, gcol_v, o_v, one, sems, xa_v):
    one[0] = 1

    def region(fn):
        pl.when(one[0] == 1)(fn)

    ffn_copies = [
        pltpu.make_async_copy(src, dst, sems.at[10 + j])
        for j, (src, dst) in enumerate(
            [(wg_hbm, wg_v), (wu_hbm, wu_v), (wo_hbm, wo_v), (wd_hbm, wd_v)])]

    def attention(qt_v, k_v, kb_v, vt_v, p_v, l_v, ot_v, unsafe_v):
        def query_block(n):
            return (n // H + 2) % 4

        def keys(c, lo=KC, hi=KC):
            return jnp.concatenate(
                [k_v[pl.ds(c * KM, KM), :]]
                + [k_v[pl.ds(KV0 + c * KV + a - KM, b - a), :]
                   for a, b in ((KM, lo), (hi, KC)) if b > a], axis=0)

        def key_columns(k):
            k = k.astype(F32)
            return [jnp.broadcast_to(k[:, d:d + 1], (k.shape[0], 128)) for d in range(DH)]

        def weights(n, u, first):
            head = pl.multiple_of(n % H * DH, G * DH) + u * DH
            qt = qt_v[query_block(n), pl.ds(head, DH), :]
            t0 = u % 4
            qf = qt[:, t0 * 128:(t0 + 1) * 128].astype(F32)
            qd = [jnp.broadcast_to(qf[d:d + 1], (8, 128)) for d in range(DH)]
            l = [None] * 4
            for c in range(NKC):
                inside = 0 < c < NKC - 1
                lo, hi = KM if inside and not first else KC - 16, KC
                fill = first and inside and u >= 4 and c % 4 == t0
                if fill:
                    lo, hi = KM, KM + 16
                    cols = key_columns(k_v[pl.ds(KV0 + c * KV, 16), :])
                    for d in range(DH):
                        kb_v[d, pl.ds(c * KV, 16)] = cols[d]
                rows = []
                for t in range(4):
                    k = keys(c, lo, hi) if t == t0 else keys(c)
                    p = jnp.exp2(_dot(k, qt[:, t * 128:(t + 1) * 128]))
                    rows.append([p[r:r + 8] for r in range(0, p.shape[0], 8)])
                extra = []
                for r in range(lo - KM, hi - KM, 8):
                    kd = [cols[d][r:r + 8] if fill else kb_v[d, pl.ds(c * KV + r, 8)]
                          for d in range(DH)]
                    extra.append(jnp.exp2(functools.reduce(
                        jnp.add, [qd[d] * kd[d] for d in range(DH)])))
                tiles = [r[:lo // 8] + extra + r[lo // 8:] if t == t0 else r
                         for t, r in enumerate(rows)]
                p_v[u, pl.ds(c * KC, KC), :] = jnp.concatenate(
                    [jnp.concatenate(r, axis=0) for r in tiles], axis=1).astype(BF16)
                for z, e in enumerate(extra):
                    r = len(rows[t0]) * z // len(extra) + 1
                    rows[t0][r] = rows[t0][r] + e
                for t in range(4):
                    if c > 0:
                        rows[t][0] = rows[t][0] + l[t]
                    l[t] = _tree_sum(rows[t])
                if c == NKC - 1:
                    l_v[u] = jnp.concatenate(l, axis=1)
                yield

        def store_heads(t, slot):
            o_v[t % HT, query_block(4 * t)] = ot_v[slot].T

        def outputs(n, u):
            if u % 4 == 0:
                store_heads(jnp.maximum(n // 4 + u // 4 - 1, 0), (u // 4 + 1) % 2)
            l = jnp.sum(l_v[u], axis=0, keepdims=True)
            for c in range(NKC):
                p = p_v[u, pl.ds(c * KC, KC), :]
                yield
                o = _dot(vt_v[c], p)
                acc = o if c == 0 else acc + o
                if c == NKC - 1:
                    g = grow_v[query_block(n)][:1]
                    ot_v[u // 4, pl.ds(u % 4 * DH, DH), :] = acc * (g / l)
                    in_range = jnp.logical_and(l >= L_MIN, l <= L_MAX)
                    unsafe_v[...] = jnp.where(in_range, unsafe_v[...], 1.0)
                yield

        def step(n, do_outputs=True, do_weights=True):
            outs = itertools.chain(*[outputs(n, u) for u in range(G) if do_outputs])
            news = itertools.chain(*[weights(n + G, u, not do_outputs)
                                     for u in range(G) if do_weights])
            for _ in range(G * NKC):
                next(outs, None)
                next(news, None)
                next(outs, None)

        def stripe_with_max(n, _):
            qt = qt_v[query_block(n), pl.ds(pl.multiple_of(n % H * DH, DH), DH), :]

            def tile(c, carry):
                m, l, acc = carry
                k = jnp.concatenate(
                    [k_v[pl.ds(pl.multiple_of(c * KM, 16), KM), :],
                     k_v[pl.ds(pl.multiple_of(KV0 + c * KV, 16), KV), :]], axis=0)
                s = _dot(k, qt)
                m_new = jnp.maximum(m, jnp.max(s, axis=0, keepdims=True))
                alpha = jnp.exp2(m - m_new)
                p = jnp.exp2(s - m_new)
                return (m_new, alpha * l + jnp.sum(p, axis=0, keepdims=True),
                        alpha * acc + _dot(vt_v[c], p.astype(BF16)))

            _, l, acc = lax.fori_loop(
                0, NKC, tile,
                (jnp.full((1, W), jnp.finfo(F32).min, F32), jnp.zeros((1, W), F32),
                 jnp.zeros((DH, W), F32)))
            head = pl.multiple_of(n % 4 * DH, DH)
            ot_v[0, pl.ds(head, DH), :] = acc * (grow_v[query_block(n)][:1] / l)
            pl.when(n % 4 == 3)(lambda: store_heads(n // 4, 0))

        def project(x_v, xf_v, wq_v, wt_v, gw_v, vf_v, acc_v, early_v):
            def copy(src, dst, idx, sem):
                return pltpu.make_async_copy(src.at[idx], dst.at[idx], sems.at[sem])

            top = pl.ds(0, 2 * W)
            left, right = (top, pl.ds(0, D // 2)), (top, pl.ds(D // 2, D // 2))
            small = [
                pltpu.make_async_copy(wkt_hbm, wt_v.at[pl.ds(0, DH)], sems.at[0]),
                pltpu.make_async_copy(wvt_hbm, wt_v.at[pl.ds(DH, DH)], sems.at[1]),
                pltpu.make_async_copy(gw_hbm, gw_v, sems.at[2]),
            ]
            x3, x2, x_left, x_right = [
                copy(x_hbm, x_v, idx, 3 + j)
                for j, idx in enumerate([pl.ds(3 * W, W), pl.ds(2 * W, W), left, right])]
            wq0, wq1, wq23 = [
                copy(wq_hbm, wq_v, (slice(None), pl.ds(c0, cn)), 7 + j)
                for j, (c0, cn) in enumerate([(0, 256), (256, 256), (512, 512)])]
            for cp in small + [x3, wq0, x2, wq1, x_left, wq23, x_right]:
                cp.start()
            ot_v[1] = jnp.zeros(ot_v.shape[1:], F32)
            unsafe_v[...] = jnp.zeros(unsafe_v.shape, F32)
            for cp in small:
                cp.wait()
            gw = gw_v[...].astype(F32)
            for j in range(D // 128):
                wt_v[pl.ds(2 * DH, 16), pl.ds(j * 128, 128)] = jnp.broadcast_to(
                    gw[j:j + 1, :], (16, 128)).astype(BF16)

            def widen(idx):
                xf_v[idx] = x_v[idx].astype(F32)

            def k_v_gate(i):
                rows = pl.ds(i * W, W)
                r = lax.dot_general(wt_v[...], x_v[rows, :], (((1,), (1,)), ((), ())),
                                    preferred_element_type=F32)
                vf_v[:, rows] = r[DH:2 * DH]
                kt = jnp.concatenate([r[:DH], jnp.zeros((128 - DH, W), F32)], axis=0)
                k_v[rows, :] = kt.T[:, :DH].astype(BF16)
                v_peak = jnp.max(jnp.abs(r[DH:2 * DH]), axis=0, keepdims=True)
                unsafe_v[...] = jnp.where(v_peak <= V_MAX, unsafe_v[...], 1.0)
                g = jax.nn.sigmoid(r[2 * DH:2 * DH + 8])
                grow_v[i] = g
                gcol_v[i] = jnp.broadcast_to(1.0 - g[:1], (128, W)).T

            def new_product(p, q):
                a = _operand(SU, p, q,
                             lambda i, k: xf_v[pl.ds(i * W, W), pl.ds(k * 256, 256)])
                xa_v[7 * p + q] = a
                return _dot(a, _operand(
                    SV, p, q, lambda k, j: wq_v[pl.ds(k * 256, 256), pl.ds(j * 256, 256)]))

            early = [(1, 1), (1, 3), (3, 1), (3, 3)]

            def product(p, q):
                if (p, q) in early:
                    return early_v[early.index((p, q))]
                return new_product(p, q)

            def emit(i, j, v):
                scale = DH ** -0.5 * math.log2(math.e)
                qt_v[i, pl.ds(j * 256, 256), :] = (v.T * scale).astype(BF16)

            x3.wait()
            widen(pl.ds(3 * W, W))
            k_v_gate(3)
            wq0.wait()

            @region
            def _():
                for j, (p, q) in enumerate(early):
                    early_v[j] = new_product(p, q)

            @region
            def _():
                cols = key_columns(jnp.concatenate(
                    [k_v[pl.ds(KV0 + c * KV + 16, 16), :] for c in range(NKC)], axis=0))
                for d in range(DH):
                    for c in range(NKC):
                        kb_v[d, pl.ds(c * KV + 16, 16)] = cols[d][c * 16:(c + 1) * 16]

            x2.wait()
            wq1.wait()

            @region
            def _():
                widen(pl.ds(2 * W, W))
                k_v_gate(2)
                _strassen2(OUTER[:2], product, emit, acc_v)

            x_left.wait()
            wq23.wait()

            @region
            def _():
                widen(left)
                _strassen2(OUTER[2:4], product, emit, acc_v)

            x_right.wait()

            @region
            def _():
                widen(right)
                k_v_gate(0)
                k_v_gate(1)
                for c in range(NKC):
                    vt_v[c] = jnp.concatenate(
                        [vf_v[:, c * KM:(c + 1) * KM],
                         vf_v[:, KV0 + c * KV:KV0 + (c + 1) * KV]], axis=1).astype(BF16)
                _strassen2(OUTER[4:], product, emit, acc_v)

        pl.run_scoped(
            project, pltpu.VMEM((S, D), BF16), pltpu.VMEM((S, D), F32),
            pltpu.VMEM((D, D), BF16), pltpu.VMEM((2 * DH + 16, D), BF16),
            pltpu.VMEM((8, 128), BF16), pltpu.VMEM((DH, S), F32),
            pltpu.VMEM((4, 4, W, 256), F32), pltpu.VMEM((4, W, 256), F32))

        def body(i, _):
            @pl.when(i == 2)
            def _():
                for cp in ffn_copies:
                    cp.start()

            step(i * G)

        last = 4 * H // G - 1
        region(lambda: step(-G, do_outputs=False))
        lax.fori_loop(0, last, body, None)
        step(last * G, do_weights=False)
        store_heads(4 * HT - 1, 1)

        @pl.when(jnp.max(unsafe_v[...]) > 0.0)
        def _():
            lax.fori_loop(0, 4 * H, stripe_with_max, None)

    pl.run_scoped(
        attention, pltpu.VMEM((4, D, W), BF16), pltpu.VMEM((S, DH), BF16),
        pltpu.VMEM((DH, S - KV0, 128), F32), pltpu.VMEM((NKC, DH, KC), BF16),
        pltpu.VMEM((G, S, W), BF16), pltpu.VMEM((G, 8, W), F32),
        pltpu.VMEM((2, 128, W), F32), pltpu.VMEM((1, W), F32))

    def ffn(h_v, acc_v):
        def up_chunk(c, _):
            c0 = pl.multiple_of(c * 512, 512)

            def wblock(k, j):
                idx = pl.ds(k * 256, 256), pl.ds(c0 + j * 128, 128)
                return jnp.concatenate([wg_v[idx], wu_v[idx]], axis=1)

            def emit(i, j, v):
                h_v[4 * c + j, i] = jnp.maximum(v[:, :128], 0.0) * v[:, 128:] * gcol_v[i]

            _strassen2(OUTER_UP,
                       lambda p, q: _dot(xa_v[7 * p + q], _operand(SV, p, q, wblock)),
                       emit, None, OUTER_UP, INNER_UP)

        for cp in ffn_copies:
            cp.wait()
        lax.fori_loop(0, NCH, up_chunk, None)

        def hblock(i, k):
            return jnp.concatenate(
                [h_v[4 * t + k, i] for t in range(NCH)]
                + [o_v[4 * t + k, i] for t in range(D // 512)], axis=1)

        def wblock(k, j):
            cs = pl.ds(j * 256, 256)
            return jnp.concatenate(
                [wd_v[pl.ds((4 * t + k) * 128, 128), cs] for t in range(NCH)]
                + [wo_v[pl.ds((4 * t + k) * 128, 128), cs] for t in range(D // 512)],
                axis=0)

        def product(p, q):
            return _dot(_operand(SU, p, q, hblock), _operand(SV, p, q, wblock))

        def staging(i, j):
            return wg_v.at[pl.ds(i % 2 * W, W), pl.ds(i // 2 * D + j * 256, 256)]

        def emit(i, j, v):
            staging(i, j)[...] = v.astype(BF16)

        def out_copy(i, j):
            return pltpu.make_async_copy(
                staging(i, j), out_hbm.at[pl.ds(i * W, W), pl.ds(j * 256, 256)],
                sems.at[14 + 4 * i + j])

        blocks = [(i, j) for i in range(4) for j in range(4)]

        @region
        def _():
            for p in OUTER[:-1]:
                _strassen2((p,), product, emit, acc_v)
            for i, j in blocks:
                if (i, j) not in QUADS:
                    out_copy(i, j).start()

        @region
        def _():
            prods = {q: product(OUTER[-1], q) for q in INNER[:-1]}
            for i, j in QUADS:
                v = _signed_sum([(1, acc_v[i, j])] + [
                    (SW[q][i, j], m) for q, m in prods.items() if (i, j) in SW[q]])
                if (i, j) == (0, 0):
                    acc_v[i, j] = v
                else:
                    emit(i, j, v)
            for i, j in QUADS[:-1]:
                out_copy(i, j).start()

        @region
        def _():
            emit(0, 0, acc_v[0, 0] + product(OUTER[-1], INNER[-1]))
            out_copy(0, 0).start()

        for i, j in blocks:
            out_copy(i, j).wait()

    pl.run_scoped(ffn, pltpu.VMEM((4 * NCH, 4, W, 128), F32),
                  pltpu.VMEM((4, 4, W, 256), F32))


def _entry(*refs):
    pl.run_scoped(functools.partial(_kernel, *refs),
                  pltpu.VMEM((49, W, D // 4), BF16))


@jax.jit
def pallas_gated_mix__grouped_kv_mqa__glu_gated_reglu__prompt_kernel(
    A_x: jax.Array,
    A_wq: jax.Array,
    A_wk: jax.Array,
    A_wv: jax.Array,
    A_wo: jax.Array,
    B_x: jax.Array,
    B_W_gate: jax.Array,
    B_W_up: jax.Array,
    B_W_down: jax.Array,
    gate_w: jax.Array,
):
    del B_x
    any_spec = pl.BlockSpec(memory_space=pl.ANY)
    out = pl.pallas_call(
        _entry,
        out_shape=jax.ShapeDtypeStruct((S, D), BF16),
        in_specs=[any_spec] * 9,
        out_specs=any_spec,
        scratch_shapes=[
            pltpu.VMEM((D, D), BF16),
            pltpu.VMEM((D, F), BF16),
            pltpu.VMEM((D, F), BF16),
            pltpu.VMEM((F, D), BF16),
            pltpu.VMEM((4, 8, W), F32),
            pltpu.VMEM((4, W, 128), F32),
            pltpu.VMEM((HT, 4, W, 128), F32),
            pltpu.SMEM((1,), jnp.int32),
            pltpu.SemaphoreType.DMA((30,)),
        ],
        compiler_params=pltpu.CompilerParams(vmem_limit_bytes=127 * 2**20),
        name="gated_mix",
    )(
        A_x.reshape(S, D), A_wq, A_wk.T, A_wv.T, A_wo, B_W_gate, B_W_up, B_W_down,
        gate_w.reshape(8, 128),
    )
    return out.reshape(1, S, D)
```

```python
import functools
import itertools
import math

import jax
import jax.numpy as jnp
from jax import lax
from jax.experimental import pallas as pl
from jax.experimental.pallas import tpu as pltpu

F32 = jnp.float32
BF16 = jnp.bfloat16

S = 2048
D = 1024
H = 32
DH = 32
F = 3584

W = S // 4
G = 8
KC = 128
NKC = S // KC
KV = 32
KM = KC - KV
KV0 = NKC * KM
HT = D // 128
NCH = F // 512

L_MIN, L_MAX, V_MAX = 2.0 ** -20, 2.0 ** 40, 2.0 ** 80

SU = ({(0, 0): 1, (1, 1): -1}, {(1, 0): 1, (1, 1): -1}, {(0, 0): 1}, {(1, 1): 1},
      {(0, 1): 1, (0, 0): -1}, {(1, 0): 1, (0, 0): -1}, {(0, 1): 1, (1, 1): -1})
SV = ({(0, 0): 1, (1, 1): -1}, {(0, 0): 1}, {(0, 1): 1, (1, 1): 1},
      {(1, 0): 1, (0, 0): 1}, {(1, 1): 1}, {(0, 0): 1, (0, 1): 1},
      {(1, 0): 1, (1, 1): 1})
SW = ({(0, 0): 1, (1, 1): 1}, {(1, 0): 1, (1, 1): -1}, {(0, 1): 1, (1, 1): 1},
      {(0, 0): 1, (1, 0): 1}, {(0, 0): -1, (0, 1): 1}, {(1, 1): 1}, {(0, 0): 1})
QUADS = ((1, 0), (0, 1), (1, 1), (0, 0))
OUTER, INNER = (1, 3, 0, 2, 4, 5, 6), (1, 0, 2, 4, 3, 5, 6)
OUTER_UP, INNER_UP = (1, 5, 3, 0, 2, 4, 6), (1, 2, 3, 4, 0, 5, 6)
INNER_DOWN = (4, 0, 1, 2, 3, 5, 6)


def _dot(a, b):
    return jnp.dot(a, b, preferred_element_type=F32)


def _tree_sum(xs):
    while len(xs) > 1:
        xs = [functools.reduce(jnp.add, xs[i:i + 2]) for i in range(0, len(xs), 2)]
    return xs[0]


def _signed_sum(terms):
    terms = sorted(terms, key=lambda t: -t[0])
    acc = terms[0][1] if terms[0][0] > 0 else -terms[0][1]
    for sign, v in terms[1:]:
        acc = acc + v if sign > 0 else acc - v
    return acc


def _operand(table, p, q, block, swap=False):
    terms = [(s * t, block(2 * a + c, 2 * b + d))
             for (a, b), s in table[p].items() for (c, d), t in table[q].items()]
    if len(terms) == 1:
        return terms[0][1].astype(BF16)
    if swap and len(terms) == 4:
        terms[1], terms[2] = terms[2], terms[1]
    return _signed_sum([(s, v.astype(F32)) for s, v in terms]).astype(BF16)


def _strassen2(part, product, emit, acc_ref=None, outer=OUTER, inner=INNER):
    before = outer[:outer.index(part[0])]

    def total(i, j, terms):
        if any((i // 2, j // 2) in SW[r] for r in before):
            terms = [(1, acc_ref[i, j])] + terms
        return _signed_sum(terms)

    pending = {}
    for n, p in enumerate(part):
        prods = {q: product(p, q) for q in inner}
        later = outer[len(before) + n + 1:]
        for i2, j2 in QUADS:
            v = _signed_sum([(SW[q][i2, j2], m) for q, m in prods.items()
                             if (i2, j2) in SW[q]])
            for (i1, j1), sign in SW[p].items():
                i, j = 2 * i1 + i2, 2 * j1 + j2
                pending.setdefault((i, j), []).append((sign, v))
                if not any((i1, j1) in SW[r] for r in later):
                    emit(i, j, total(i, j, pending.pop((i, j))))
    for (i, j), terms in pending.items():
        acc_ref[i, j] = total(i, j, terms)


def _kernel(x_hbm, wq_hbm, wkt_hbm, wvt_hbm, wo_hbm, wg_hbm, wu_hbm, wd_hbm, gw_hbm,
            out_hbm, wo_v, wg_v, wu_v, wd_v, grow_v, gcol_v, o_v, one, sems, xa_v):
    one[0] = 1

    def region(fn):
        pl.when(one[0] == 1)(fn)

    ffn_copies = [
        pltpu.make_async_copy(src, dst, sems.at[10 + j])
        for j, (src, dst) in enumerate(
            [(wg_hbm, wg_v), (wu_hbm, wu_v), (wo_hbm, wo_v), (wd_hbm, wd_v)])]

    def attention(qt_v, k_v, kb_v, vt_v, p_v, l_v, ot_v, unsafe_v):
        def query_block(n):
            return (n // H + 2) % 4

        def keys(c, lo=KC, hi=KC):
            return jnp.concatenate(
                [k_v[pl.ds(c * KM, KM), :]]
                + [k_v[pl.ds(KV0 + c * KV + a - KM, b - a), :]
                   for a, b in ((KM, lo), (hi, KC)) if b > a], axis=0)

        def key_columns(k):
            k = k.astype(F32)
            return [jnp.broadcast_to(k[:, d:d + 1], (k.shape[0], 128)) for d in range(DH)]

        def weights(n, u, first):
            head = pl.multiple_of(n % H * DH, G * DH) + u * DH
            qt = qt_v[query_block(n), pl.ds(head, DH), :]
            t0 = u % 4
            qf = qt[:, t0 * 128:(t0 + 1) * 128].astype(F32)
            qd = [jnp.broadcast_to(qf[d:d + 1], (8, 128)) for d in range(DH)]
            l = [None] * 4
            for c in range(NKC):
                lo, hi = KC - 16 if first or c == NKC - 1 else KM, KC
                fill = first and u >= 4 and c % 4 == t0 and c < NKC - 1
                if fill:
                    lo, hi = KM, KM + 16
                    cols = key_columns(k_v[pl.ds(KV0 + c * KV, 16), :])
                    for d in range(DH):
                        kb_v[d, pl.ds(c * KV, 16)] = cols[d]
                rows = []
                for t in range(4):
                    k = keys(c, lo, hi) if t == t0 else keys(c)
                    p = jnp.exp2(_dot(k, qt[:, t * 128:(t + 1) * 128]))
                    rows.append([p[r:r + 8] for r in range(0, p.shape[0], 8)])
                extra = []
                for r in range(lo - KM, hi - KM, 8):
                    kd = [cols[d][r:r + 8] if fill else kb_v[d, pl.ds(c * KV + r, 8)]
                          for d in range(DH)]
                    extra.append(jnp.exp2(functools.reduce(
                        jnp.add, [qd[d] * kd[d] for d in range(DH)])))
                tiles = [r[:lo // 8] + extra + r[lo // 8:] if t == t0 else r
                         for t, r in enumerate(rows)]
                p_v[u, pl.ds(c * KC, KC), :] = jnp.concatenate(
                    [jnp.concatenate(r, axis=0) for r in tiles], axis=1).astype(BF16)
                for z, e in enumerate(extra):
                    r = len(rows[t0]) * z // len(extra) + 1 + z // 2
                    rows[t0][r] = rows[t0][r] + e
                for t in range(4):
                    if c > 0:
                        rows[t][0] = rows[t][0] + l[t]
                    l[t] = _tree_sum(rows[t])
                if c == NKC - 1:
                    l_v[u] = jnp.concatenate(l, axis=1)
                yield

        def store_heads(t, slot):
            o_v[t % HT, query_block(4 * t)] = ot_v[slot].T

        def outputs(n, u):
            if u % 4 == 0:
                store_heads(jnp.maximum(n // 4 + u // 4 - 1, 0), (u // 4 + 1) % 2)
            l = jnp.sum(l_v[u], axis=0, keepdims=True)
            for c in range(NKC):
                o = _dot(vt_v[c], p_v[u, pl.ds(c * KC, KC), :])
                acc = o if c == 0 else acc + o
                if c == NKC - 1:
                    g = grow_v[query_block(n)][:1]
                    ot_v[u // 4, pl.ds(u % 4 * DH, DH), :] = acc * (
                        g * pl.reciprocal(l, full_range=False))
                    in_range = jnp.logical_and(l >= L_MIN, l <= L_MAX)
                    unsafe_v[...] = jnp.where(in_range, unsafe_v[...], 1.0)
                yield

        def step(n, do_outputs=True, do_weights=True):
            outs = itertools.chain(*[outputs(n, u) for u in range(G) if do_outputs])
            news = itertools.chain(*[weights(n + G, u, not do_outputs)
                                     for u in range(G) if do_weights])
            for _ in range(G * NKC):
                next(outs, None)
                next(news, None)

        def stripe_with_max(n, _):
            qt = qt_v[query_block(n), pl.ds(pl.multiple_of(n % H * DH, DH), DH), :]

            def tile(c, carry):
                m, l, acc = carry
                k = jnp.concatenate(
                    [k_v[pl.ds(pl.multiple_of(c * KM, 16), KM), :],
                     k_v[pl.ds(pl.multiple_of(KV0 + c * KV, 16), KV), :]], axis=0)
                s = _dot(k, qt)
                m_new = jnp.maximum(m, jnp.max(s, axis=0, keepdims=True))
                alpha = jnp.exp2(m - m_new)
                p = jnp.exp2(s - m_new)
                return (m_new, alpha * l + jnp.sum(p, axis=0, keepdims=True),
                        alpha * acc + _dot(vt_v[c], p.astype(BF16)))

            _, l, acc = lax.fori_loop(
                0, NKC, tile,
                (jnp.full((1, W), jnp.finfo(F32).min, F32), jnp.zeros((1, W), F32),
                 jnp.zeros((DH, W), F32)))
            head = pl.multiple_of(n % 4 * DH, DH)
            ot_v[0, pl.ds(head, DH), :] = acc * (grow_v[query_block(n)][:1] / l)
            pl.when(n % 4 == 3)(lambda: store_heads(n // 4, 0))

        def project(x_v, xf_v, wq_v, wt_v, wf_v, gw_v, vf_v, acc_v, early_v):
            def copy(src, dst, idx, sem):
                return pltpu.make_async_copy(src.at[idx], dst.at[idx], sems.at[sem])

            top = pl.ds(0, 2 * W)
            left, right = (top, pl.ds(0, D // 2)), (top, pl.ds(D // 2, D // 2))
            small = [
                pltpu.make_async_copy(wkt_hbm, wt_v.at[pl.ds(0, DH)], sems.at[0]),
                pltpu.make_async_copy(wvt_hbm, wt_v.at[pl.ds(DH, DH)], sems.at[1]),
                pltpu.make_async_copy(gw_hbm, gw_v, sems.at[2]),
            ]
            x3, x2, x_left, x_right = [
                copy(x_hbm, x_v, idx, 3 + j)
                for j, idx in enumerate([pl.ds(3 * W, W), pl.ds(2 * W, W), left, right])]
            wq0, wq1, wq23 = [
                copy(wq_hbm, wq_v, (slice(None), pl.ds(c0, cn)), 7 + j)
                for j, (c0, cn) in enumerate([(0, 256), (256, 256), (512, 512)])]
            for cp in small + [x3, wq0, x2, wq1, x_left, wq23, x_right]:
                cp.start()
            ot_v[1] = jnp.zeros(ot_v.shape[1:], F32)
            unsafe_v[...] = jnp.zeros(unsafe_v.shape, F32)
            for cp in small:
                cp.wait()
            gw = gw_v[...].astype(F32)
            wf_v[pl.ds(0, 2 * DH), :] = wt_v[...].astype(F32)
            for j in range(D // 128):
                wf_v[pl.ds(2 * DH, 8), pl.ds(j * 128, 128)] = jnp.broadcast_to(
                    gw[j:j + 1, :], (8, 128))

            def widen(idx):
                xf_v[idx] = x_v[idx].astype(F32)

            def k_v_gate(i):
                rows = pl.ds(i * W, W)
                r = lax.dot_general(wf_v[...], x_v[rows, :], (((1,), (1,)), ((), ())),
                                    preferred_element_type=F32)
                vf_v[:, rows] = r[DH:2 * DH]
                kt = jnp.concatenate([r[:DH], jnp.zeros((128 - DH, W), F32)], axis=0)
                k_v[rows, :] = kt.T[:, :DH].astype(BF16)
                v_peak = jnp.max(jnp.abs(r[DH:2 * DH]), axis=0, keepdims=True)
                unsafe_v[...] = jnp.where(v_peak <= V_MAX, unsafe_v[...], 1.0)
                g = jax.nn.sigmoid(r[2 * DH:2 * DH + 8])
                grow_v[i] = g
                gcol_v[i] = jnp.broadcast_to(1.0 - g[:1], (128, W)).T

            def new_product(p, q):
                a = _operand(SU, p, q,
                             lambda i, k: xf_v[pl.ds(i * W, W), pl.ds(k * 256, 256)])
                xa_v[7 * p + q] = a
                return _dot(a, _operand(
                    SV, p, q, lambda k, j: wq_v[pl.ds(k * 256, 256), pl.ds(j * 256, 256)]))

            early = [(1, 1), (1, 3), (3, 1), (3, 3)]

            def product(p, q):
                if (p, q) in early:
                    return early_v[early.index((p, q))]
                return new_product(p, q)

            def emit(i, j, v):
                scale = DH ** -0.5 * math.log2(math.e)
                qt_v[i, pl.ds(j * 256, 256), :] = (v.T * scale).astype(BF16)

            x3.wait()
            widen(pl.ds(3 * W, W))
            k_v_gate(3)
            wq0.wait()

            @region
            def _():
                for j, (p, q) in enumerate(early):
                    early_v[j] = new_product(p, q)

            @region
            def _():
                cols = key_columns(jnp.concatenate(
                    [k_v[pl.ds(KV0 + c * KV + 16, 16), :] for c in range(NKC)], axis=0))
                for d in range(DH):
                    for c in range(NKC):
                        kb_v[d, pl.ds(c * KV + 16, 16)] = cols[d][c * 16:(c + 1) * 16]

            x2.wait()
            wq1.wait()

            @region
            def _():
                widen(pl.ds(2 * W, W))
                k_v_gate(2)
                _strassen2(OUTER[:2], product, emit, acc_v)

            x_left.wait()
            wq23.wait()

            @region
            def _():
                widen(left)
                _strassen2(OUTER[2:4], product, emit, acc_v)

            x_right.wait()

            @region
            def _():
                widen(right)
                k_v_gate(0)
                k_v_gate(1)
                for c in range(NKC):
                    vt_v[c] = jnp.concatenate(
                        [vf_v[:, c * KM:(c + 1) * KM],
                         vf_v[:, KV0 + c * KV:KV0 + (c + 1) * KV]], axis=1).astype(BF16)
                _strassen2(OUTER[4:], product, emit, acc_v)

        pl.run_scoped(
            project, pltpu.VMEM((S, D), BF16), pltpu.VMEM((S, D), F32),
            pltpu.VMEM((D, D), BF16), pltpu.VMEM((2 * DH, D), BF16),
            pltpu.VMEM((2 * DH + 8, D), F32),
            pltpu.VMEM((8, 128), BF16), pltpu.VMEM((DH, S), F32),
            pltpu.VMEM((4, 4, W, 256), F32), pltpu.VMEM((4, W, 256), F32))

        def body(i, _):
            @pl.when(i == 2)
            def _():
                for cp in ffn_copies:
                    cp.start()

            step(i * G)

        last = 4 * H // G - 1
        region(lambda: step(-G, do_outputs=False))
        lax.fori_loop(0, last, body, None)
        step(last * G, do_weights=False)
        store_heads(4 * HT - 1, 1)

        @pl.when(jnp.max(unsafe_v[...]) > 0.0)
        def _():
            lax.fori_loop(0, 4 * H, stripe_with_max, None)

    pl.run_scoped(
        attention, pltpu.VMEM((4, D, W), BF16), pltpu.VMEM((S, DH), BF16),
        pltpu.VMEM((DH, S - KV0, 128), F32), pltpu.VMEM((NKC, DH, KC), BF16),
        pltpu.VMEM((G, S, W), BF16), pltpu.VMEM((G, 8, W), F32),
        pltpu.VMEM((2, 128, W), F32), pltpu.VMEM((1, W), F32))

    def ffn(h_v, acc_v):
        def up_chunk(c, _):
            c0 = pl.multiple_of(c * 512, 512)

            def wblock(k, j):
                idx = pl.ds(k * 256, 256), pl.ds(c0 + j * 128, 128)
                return jnp.concatenate([wg_v[idx], wu_v[idx]], axis=1)

            def emit(i, j, v):
                h_v[4 * c + j, i] = jnp.maximum(v[:, :128], 0.0) * v[:, 128:] * gcol_v[i]

            def product(p, q):
                return _dot(xa_v[7 * p + q], _operand(SV, p, q, wblock, swap=True))

            _strassen2(OUTER_UP, product, emit, None, OUTER_UP, INNER_UP)

        for cp in ffn_copies:
            cp.wait()
        lax.fori_loop(0, NCH, up_chunk, None)

        def hblock(i, k):
            return jnp.concatenate(
                [h_v[4 * t + k, i] for t in range(NCH)]
                + [o_v[4 * t + k, i] for t in range(D // 512)], axis=1)

        def wblock(k, j):
            cs = pl.ds(j * 256, 256)
            return jnp.concatenate(
                [wd_v[pl.ds((4 * t + k) * 128, 128), cs] for t in range(NCH)]
                + [wo_v[pl.ds((4 * t + k) * 128, 128), cs] for t in range(D // 512)],
                axis=0)

        def product(p, q):
            return _dot(_operand(SU, p, q, hblock), _operand(SV, p, q, wblock))

        def staging(i, j):
            return wg_v.at[pl.ds(i % 2 * W, W), pl.ds(i // 2 * D + j * 256, 256)]

        def emit(i, j, v):
            staging(i, j)[...] = v.astype(BF16)

        def out_copy(i, j):
            return pltpu.make_async_copy(
                staging(i, j), out_hbm.at[pl.ds(i * W, W), pl.ds(j * 256, 256)],
                sems.at[14 + 4 * i + j])

        blocks = [(i, j) for i in range(4) for j in range(4)]

        @region
        def _():
            for p in OUTER[:-1]:
                _strassen2((p,), product, emit, acc_v, inner=INNER_DOWN)
            for i, j in blocks:
                if (i, j) not in QUADS:
                    out_copy(i, j).start()

        @region
        def _():
            prods = {q: product(OUTER[-1], q) for q in INNER_DOWN[:-1]}
            for i, j in QUADS:
                v = _signed_sum([(1, acc_v[i, j])] + [
                    (SW[q][i, j], m) for q, m in prods.items() if (i, j) in SW[q]])
                if (i, j) == (0, 0):
                    acc_v[i, j] = v
                else:
                    emit(i, j, v)
            for i, j in QUADS[:-1]:
                out_copy(i, j).start()

        @region
        def _():
            emit(0, 0, acc_v[0, 0] + product(OUTER[-1], INNER_DOWN[-1]))
            out_copy(0, 0).start()

        for i, j in blocks:
            out_copy(i, j).wait()

    pl.run_scoped(ffn, pltpu.VMEM((4 * NCH, 4, W, 128), F32),
                  pltpu.VMEM((4, 4, W, 256), F32))


def _entry(*refs):
    pl.run_scoped(functools.partial(_kernel, *refs),
                  pltpu.VMEM((49, W, D // 4), BF16))


@jax.jit
def pallas_gated_mix__grouped_kv_mqa__glu_gated_reglu__prompt_kernel(
    A_x: jax.Array,
    A_wq: jax.Array,
    A_wk: jax.Array,
    A_wv: jax.Array,
    A_wo: jax.Array,
    B_x: jax.Array,
    B_W_gate: jax.Array,
    B_W_up: jax.Array,
    B_W_down: jax.Array,
    gate_w: jax.Array,
):
    del B_x
    any_spec = pl.BlockSpec(memory_space=pl.ANY)
    out = pl.pallas_call(
        _entry,
        out_shape=jax.ShapeDtypeStruct((S, D), BF16),
        in_specs=[any_spec] * 9,
        out_specs=any_spec,
        scratch_shapes=[
            pltpu.VMEM((D, D), BF16),
            pltpu.VMEM((D, F), BF16),
            pltpu.VMEM((D, F), BF16),
            pltpu.VMEM((F, D), BF16),
            pltpu.VMEM((4, 8, W), F32),
            pltpu.VMEM((4, W, 128), F32),
            pltpu.VMEM((HT, 4, W, 128), F32),
            pltpu.SMEM((1,), jnp.int32),
            pltpu.SemaphoreType.DMA((30,)),
        ],
        compiler_params=pltpu.CompilerParams(vmem_limit_bytes=127 * 2**20),
        name="gated_mix",
    )(
        A_x.reshape(S, D), A_wq, A_wk.T, A_wv.T, A_wo, B_W_gate, B_W_up, B_W_down,
        gate_w.reshape(8, 128),
    )
    return out.reshape(1, S, D)
```
